```python
import jax
import jax.numpy as jnp

def _softmax(x, axis=-1):
    return jax.nn.softmax(x, axis=axis)
def _gelu(x):
    return jax.nn.gelu(x, approximate=True)
def _silu(x):
    return jax.nn.silu(x)
def _sigmoid(x):
    return jax.nn.sigmoid(x)
def _layernorm(x, axis=-1, eps=1e-5):
    m = jnp.mean(x, axis=axis, keepdims=True)
    v = jnp.var(x, axis=axis, keepdims=True)
    return (x - m) / jnp.sqrt(v + eps)
def _scatter_add(tgt, idx, src, axis=0):
    return tgt.at[idx].add(src)
def _segment_sum(src, seg, n):
    return jax.ops.segment_sum(src, seg, n)
class _Rng:
    def __init__(self, key):
        self._k = key
    def _next(self):
        self._k, sub = jax.random.split(self._k)
        return sub
    def normal(self, shape):
        return jax.random.normal(self._next(), shape, dtype=jnp.bfloat16)
    def randint(self, lo, hi, shape):
        return jax.random.randint(self._next(), shape, lo, hi, dtype=jnp.int32)
    def uniform(self, shape, lo=0.0, hi=1.0):
        return jax.random.uniform(self._next(), shape, jnp.bfloat16, lo, hi)
    def permutation(self, n):
        return jax.random.permutation(self._next(), n)


kernel_name = 'parallel_sum__linear_kernel_hedgehog__glu_gated_geglu__prompt'

def _fwd_setup_inputs():
    _rng = _Rng(jax.random.key(int.from_bytes(__import__("os").urandom(4), "little")))
    _w = (lambda a: (lambda t: t.astype(jnp.bfloat16) if jnp.issubdtype(t.dtype, jnp.floating) else t)(jnp.asarray(a)))
    def _A_setup():
        B, S, D, H = 1, 2048, 448, 16
        Dh = D // H
        return {
            "x": _w((lambda *s: _rng.normal(s) * 0.05)(B, S, D)),
            "wqkv": _w((lambda *s: _rng.normal(s) * 0.05)(D, 3 * D)),
            "w_phi": _w((lambda *s: _rng.normal(s) * 0.05)(H, Dh, Dh) * (Dh ** -0.5)),
            "wo": _w((lambda *s: _rng.normal(s) * 0.05)(D, D)),
        }
    _A_in = _A_setup()

    def _B_setup():
        B, S, Dm, Df = 1, 2048, 448, 1792
        return {
            "x": _w((lambda *s: _rng.normal(s) * 0.05)(B, S, Dm)),
            "w_gate": _w((lambda *s: _rng.normal(s) * 0.05)(Dm, Df) * (Dm ** -0.5)),
            "w_up": _w((lambda *s: _rng.normal(s) * 0.05)(Dm, Df) * (Dm ** -0.5)),
            "w_down": _w((lambda *s: _rng.normal(s) * 0.05)(Df, Dm) * (Df ** -0.5)),
        }
    _B_in = _B_setup()

    return {
        "A_x": _A_in["x"],
        "A_wqkv": _A_in["wqkv"],
        "A_w_phi": _A_in["w_phi"],
        "A_wo": _A_in["wo"],
        "B_x": _B_in["x"],
        "B_w_gate": _B_in["w_gate"],
        "B_w_up": _B_in["w_up"],
        "B_w_down": _B_in["w_down"],
    }

def _fwd_reference(A_x, A_wqkv, A_w_phi, A_wo, B_x, B_w_gate, B_w_up, B_w_down):
    def _A_ref(x, wqkv, w_phi, wo):
        B, S, D = x.shape
        H = 16; Dh = D // H
        qkv = (lambda x, *d: x.transpose(*d))((x @ wqkv).reshape(B, S, 3, H, Dh), 2, 0, 3, 1, 4)
        q, k, v = qkv[0], qkv[1], qkv[2]
        pq = jnp.einsum("bhsd,hdf->bhsf", q, w_phi)
        pk = jnp.einsum("bhsd,hdf->bhsf", k, w_phi)
        phi_q = jnp.concatenate([_softmax(pq, axis=-1), _softmax(-pq, axis=-1)], axis=-1)
        phi_k = jnp.concatenate([_softmax(pk, axis=-1), _softmax(-pk, axis=-1)], axis=-1)
        kv = jnp.einsum("bhsf,bhsd->bhfd", phi_k, v)
        z  = jnp.einsum("bhsf->bhf", phi_k)
        num = jnp.einsum("bhqf,bhfd->bhqd", phi_q, kv)
        den = jnp.einsum("bhqf,bhf->bhq", phi_q, z)[..., None] + 1e-6
        o = num / den
        return (lambda x, *d: x.transpose(*d))(o, 0, 2, 1, 3).reshape(B, S, D) @ wo

    def _B_ref(x, w_gate, w_up, w_down):
        g = jnp.einsum("bsd,df->bsf", x, w_gate)
        u = jnp.einsum("bsd,df->bsf", x, w_up)
        h = _gelu(g) * u
        return jnp.einsum("bsf,fd->bsd", h, w_down)

    x = A_x
    xn = _layernorm(x, axis=-1)
    return x + _A_ref(xn, A_wqkv, A_w_phi, A_wo) + _B_ref(xn, B_w_gate, B_w_up, B_w_down)


def setup_inputs():
    _inp = _fwd_setup_inputs()
    _gk = jax.random.fold_in(jax.random.key(int.from_bytes(__import__("os").urandom(4), "little")), 2**31 - 1)
    _shapes = [[1, 2048, 448]]
    _dtypes = ['bfloat16']
    _gks = jax.random.split(_gk, len(_shapes))
    _gs = [jax.random.normal(k, s, dtype=jnp.dtype(d)) * 0.05 for k, s, d in zip(_gks, _shapes, _dtypes)]
    _inp["grad_out"] = _gs[0]
    return _inp

def reference(A_x, A_wqkv, A_w_phi, A_wo, B_w_gate, B_w_up, B_w_down, B_x, grad_out):
    _const = dict(B_x=B_x)
    def _f(*_d):
        return _fwd_reference(**{'A_x': _d[0], 'A_wqkv': _d[1], 'A_w_phi': _d[2], 'A_wo': _d[3], 'B_w_gate': _d[4], 'B_w_up': _d[5], 'B_w_down': _d[6], **_const})
    _out, _vjp = jax.vjp(_f, A_x, A_wqkv, A_w_phi, A_wo, B_w_gate, B_w_up, B_w_down)
    _grads = _vjp(grad_out)
    _out0 = jnp.asarray(_out)
    return (_out0, *[jnp.asarray(_g) for _g in _grads])
```

```python
import functools
import math

import jax
import jax.numpy as jnp
import jax.experimental.pallas as pl
import jax.experimental.pallas.tpu as pltpu

f32, bf16, i32, u32 = jnp.float32, jnp.bfloat16, jnp.int32, jnp.uint32

S, D, H, DH, F = 2048, 448, 16, 28, 1792
TM = 512
TF = 256
NI, NJ = S // TM, F // TF
HD, HM, HF = D // 2, TM // 2, TF // 2
NC = HM // 128
NG = 8
GW = 2 * DH

NN = (((1,), (0,)), ((), ()))
NT = (((1,), (1,)), ((), ()))
C0 = math.sqrt(2.0 / math.pi)
C1 = 0.044715

BW = 2 * GW
SQ, SO, SK = (3 * NJ, 3 * NJ + 2), (3 * NJ + 1, 3 * NJ + 3), 3 * NJ + 4
NS = SK + 2
NSEM = 8


def _dot(a, b, dn=NN):
    return jax.lax.dot_general(a, b, dn, preferred_element_type=f32)


def _gelu_fb(g, u, dh):
    g2 = g * g
    t = jnp.tanh(g * (C0 + (C0 * C1) * g2))
    hp = 0.5 * t + 0.5
    ge = g * hp
    dge = hp + ge * (1.0 - t) * (C0 + (3.0 * C0 * C1) * g2)
    return ge * u, dh * u * dge, dh * ge


def _slabs(a, n):
    return [a[8 * r:8 * r + 8] for r in range(n)]


def _tree(op, xs):
    xs = list(xs)
    while len(xs) > 1:
        xs = [op(xs[k], xs[k + 1]) if k + 1 < len(xs) else xs[k] for k in range(0, len(xs), 2)]
    return xs[0]


def _head_reduce(op, slabs):
    m = _tree(op, slabs)
    m = op(m, pltpu.roll(m, 2, 0))
    return op(m, pltpu.roll(m, 4, 0))


def _dual_softmax(p):
    ps = _slabs(p, 7)
    mx = _head_reduce(jnp.maximum, ps)
    mn = _head_reduce(jnp.minimum, ps)
    ea = [jnp.exp(s - mx) for s in ps]
    eb = [jnp.exp(mn - s) for s in ps]
    ra = 1.0 / _head_reduce(jnp.add, ea)
    rb = 1.0 / _head_reduce(jnp.add, eb)
    return [e * ra for e in ea], [e * rb for e in eb]


def _dual_softmax_bwd(a, b, dphi):
    ds = _slabs(dphi, 14)
    ta = [x * d for x, d in zip(a, ds[:7])]
    tb = [x * d for x, d in zip(b, ds[7:])]
    sa = _head_reduce(jnp.add, ta)
    sb = _head_reduce(jnp.add, tb)
    return [(t1 - x * sa) - (t2 - y * sb) for t1, x, t2, y in zip(ta, a, tb, b)]


def _div(x, n):
    return (x * (65536 // n + 1)) >> 16


def _e_rows(lo, n):
    r = jax.lax.broadcasted_iota(i32, (n, DH), 0) + lo
    c = jax.lax.broadcasted_iota(i32, (n, DH), 1)
    fr = (r - GW * _div(r, GW)) >> 1
    return jnp.where(fr == c, 1.0, 0.0).astype(bf16)


def _head_match(shape, feat_axis, feat_lo, hd_lo):
    r = jax.lax.broadcasted_iota(i32, shape, feat_axis) + feat_lo
    c = jax.lax.broadcasted_iota(i32, shape, 1 - feat_axis) + hd_lo
    return (2 * _div(r, GW) + (r & 1)) == _div(c, DH)


def _kv_mask():
    r = jax.lax.broadcasted_iota(i32, (64, 2 * GW), 0)
    c = jax.lax.broadcasted_iota(i32, (64, 2 * GW), 1)
    hr = jnp.where(r < GW, jnp.where(r < DH, 0, 1), jnp.where(r < GW + 4, 0, 1))
    return hr == (c & 1)


def _pk(a):
    return pltpu.bitcast(a, u32)


def _up(a):
    return pltpu.bitcast(a, bf16)


def _blocks(z):
    r, c = z.shape[0] // 2, z.shape[1] // 2
    return z[:r, :c], z[:r, c:], z[r:, :c], z[r:, c:]


def _unblock(c11, c12, c21, c22):
    return jnp.concatenate([jnp.concatenate([c11, c12], 1), jnp.concatenate([c21, c22], 1)], 0)


def _scomb(z11, z12, z21, z22):
    return [z11 + z22, z11, z22, z11 + z12, z21 + z22, z21 - z11, z12 - z22]


def _xcomb(z11, z12, z21, z22):
    return [z11 + z22, z11, z22, z11 - z12, z22 - z21, z21 + z11, z12 + z22]


SC = ((0, 3, 1), (0,), (3,), (0, 1, 1), (2, 3, 1), (2, 0, -1), (1, 3, -1))
XC = ((0, 3, 1), (0,), (3,), (0, 1, -1), (3, 2, -1), (2, 0, 1), (1, 3, 1), (1,), (2,))


def _pick(c, z):
    return z[c[0]] if len(c) == 1 else z[c[0]] + z[c[1]] if c[2] > 0 else z[c[0]] - z[c[1]]


def _comb2(tab, z, k):
    o = [_pick(tab[k], (z[r][t], z[r][2 + t], z[2 + r][t], z[2 + r][2 + t])) for r in range(2) for t in range(2)]
    return [_pick(c, o) for c in tab]


def _post1z(p, n):
    if n == 0:
        return ((p[0] - p[6]) + p[4]) - p[3]
    if n == 3:
        return ((p[0] - p[5]) + p[1]) - p[2]
    return _post1n(p, n)


def _post_2(post, p):
    m = [post(p[k]) for k in range(7)]
    c = [post([m[k][n] for k in range(7)]) for n in range(4)]
    return [[c[2 * (r % 2) + t % 2][2 * (r // 2) + t // 2] for t in range(4)] for r in range(4)]


def _cast(ts):
    return [t.astype(bf16) for t in ts]


def _token(ts):
    ps = []
    for t in ts:
        t = pltpu.bitcast(t, u32)
        if t.shape[1] % 128:
            t = jnp.concatenate([t, jnp.zeros((t.shape[0], -t.shape[1] % 128), u32)], 1)
        ps += [t[r:r + 8, c:c + 128] for r in range(0, t.shape[0], 8) for c in range(0, t.shape[1], 128)]
    return _tree(jnp.bitwise_or, ps)


def _split(u):
    return [pltpu.unpack_elementwise(u, index=k, packed_dtype=bf16, unpacked_dtype=f32) for k in range(2)]


def _join(e, o):
    return pltpu.pack_elementwise([e, o], packed_dtype=bf16).astype(u32)


def _raw_comb(comb, z):
    es, os_ = zip(*[_split(t) for t in z])
    out = [_join(e, o) for e, o in zip(comb(*es), comb(*os_))]
    out[1], out[2] = z[0], z[3]
    return out


PA1 = ((0, 0), (6, 1), (1, 6), (2, 5), (5, 2), (3, 3), (4, 4))
PA2 = ((0, 0), (4, 1), (1, 6), (2, 5), (3, 2), (5, 3), (6, 4))
PA3 = ((0, 0), (4, 1), (1, 4), (2, 3), (3, 2), (5, 5), (6, 6))


ORD1 = (1, 3, 2, 4, 0, 5, 6)


ORD2 = (1, 3, 2, 4, 0, 5, 6)


def _post1(p):
    return (p[0] - p[3]) + (p[4] - p[6]), p[2] + p[4], p[1] + p[3], (p[0] + p[1]) - (p[2] + p[5])


FIN1 = {1: 2, 3: 1, 5: 3, 6: 0}
PIN1 = {1: 4, 3: 6}


PINI=None
QI=5
PORD=(0,3,1,2)
KORD=(1,4,0,2,3,5,6)
GS=32
ORDO=(1,3,2,4,0,5,6)
FINO={1:2,3:1,5:3,6:0}
SL=128
HOLD=2
LT=20
DL=None
GL=(None,None)
PING={1:(10,40),3:(10,40),5:(10,50),6:(30,70)}
F0W=(0,45,20)
W0=102
Y0=30
T0=14
T1=30
T2=110
AH=52
WB=9
YS=14
GA=28


def _post1n(p, n):
    if n == 0:
        return ((p[4] - p[3]) + p[0]) - p[6]
    if n == 3:
        return ((p[1] - p[2]) + p[0]) - p[5]
    return p[2] + p[4] if n == 1 else p[1] + p[3]


def _post2(m):
    return (m[0] + m[3]) + (m[6] - m[4]), m[2] + m[4], m[1] + m[3], (m[0] - m[1]) + (m[2] + m[5])


def _post3(q):
    return (q[0] - q[3]) + (q[6] - q[4]), q[2] - q[4], q[3] - q[1], (q[0] - q[1]) + (q[5] - q[2])


def _kernel(x_h, wqkv_h, wphi_h, wo_h, wg_h, wu_h, wd_h, dy_h,
            out_h, dx_h, dwqkv_h, dwphi_h, dwo_h, dwg_h, dwu_h, dwd_h,
            xr, yr, st, wraw, wn, wt, wnk, wtk, x2, y2, wn2, wt2, wd2, wdT, px2, pw2, po, px, pw, sw,
            wqkv, wphi, wo, wT, wpqT, pcs, w3, w2,
            phik, vta, kv, dkv, kvm, kvmT, dnb, lnm, pg, pa, grem, rq,
            sout, sdx, sqkv, sphi, swo, zero, sem):
    w_h = (wg_h, wu_h, wd_h)
    dw_h = (dwg_h, dwu_h, dwd_h)

    def cp(src, dst, k):
        return pltpu.make_async_copy(src, dst, sem.at[k])

    def span(i, n):
        return pl.ds(i * n if isinstance(i, int) else pl.multiple_of(i * n, n), n)

    def cp_x(i, k):
        return cp(x_h.at[:, span(i, TM)], xr.at[i], k)

    def cp_dy(i, k):
        return cp(dy_h.at[:, span(i, TM)], yr.at[i], k)

    def cp_w(j, m, k):
        return cp(w_h[m].at[:, span(j, TF)], wraw.at[3 * j + m, 0:D], k)

    def cp_dw(j):
        return [cp(sw.at[j, m, 0:D], dw_h[m].at[:, span(j, TF)], 6) for m in range(3)]

    def cp_out(i):
        return cp(sout.at[i], out_h.at[:, span(i, TM)], 6)

    def cp_dx(i):
        return cp(sdx.at[i], dx_h.at[:, span(i, TM)], 6)

    cp_datt = [cp(sqkv.at[:, a:b], dwqkv_h.at[:, a:b], 6) for a, b in ((0, 384), (2 * D, 3 * D), (384, 2 * D))]
    cp_datt += [cp(sphi, dwphi_h, 6), cp(swo, dwo_h, 6)]

    hist = []

    def mm(a, b, dn=NN):
        r = _dot(a, b, dn)
        hist.append(r)
        return r

    def ld(u, e):
        if e is None:
            return u
        return u | jnp.tile(e, (u.shape[0] // 8, -(-u.shape[1] // 128)))[:, 0:u.shape[1]]

    def lagged(jobs, lag):
        return [(job, lag) for job in jobs]

    def entry(lag):
        if lag is None or len(hist) < lag:
            return None
        return pltpu.bitcast(hist[-lag][0:8, 0:128], u32) & zero[0].astype(u32)

    def pin(u, jobs):
        if not jobs:
            return _up(u)
        ng = u.shape[0] // 8
        at = [q * ng // len(jobs) for q in range(len(jobs))]
        rows, last = [], 0
        for g in sorted(set(at)):
            if g > last:
                rows.append(u[8 * last:8 * g])
            t = u[8 * g:8 * g + 8, 0:128]
            for q, (job, lag) in enumerate(jobs):
                if at[q] == g:
                    t = t | (job(entry(lag)) & zero[0].astype(u32))[:, 0:t.shape[1]]
            rows.append(t if u.shape[1] <= 128 else jnp.concatenate([t, u[8 * g:8 * g + 8, 128:]], 1))
            last = g + 1
        if last < ng:
            rows.append(u[8 * last:])
        return _up(jnp.concatenate(rows, 0))

    def spread(host, name, jobs, lag, lo=0, hi=14):
        slots = host.setdefault(name, [[] for _ in range(14)])
        w = [2 - q % 2 for q in range(lo, hi)]
        acc = 0
        for q in range(lo, hi):
            slots[q] += lagged(jobs[len(jobs) * acc // sum(w):len(jobs) * (acc + w[q - lo]) // sum(w)], lag)
            acc += w[q - lo]

    def run(jobs):
        for job in jobs:
            job(None)

    def fuse(jobs):
        return lambda e: _token([job(e) for job in jobs])

    def quad(ref, r, c, w, e):
        return [ld(_pk(ref[p + 16 * r:p + 16 * r + 16, q + 128 * c:q + 128 * c + 128]), e) for p in (0, HD) for q in (0, w)]

    def stats_x(i):
        def job(c, e):
            cs = slice(128 * c, 128 * c + 128)
            x0 = jnp.broadcast_to(xr[i, 0:16, cs].astype(f32)[0:1], (8, 128))
            a1, a2, ts = [None] * 2, [None] * 2, []
            for r in range(D // 16):
                for q, t in enumerate(_split(ld(_pk(xr[i, 16 * r:16 * r + 16, cs]), e))):
                    t = t - x0
                    a1[q] = t if r == 0 else a1[q] + t
                    a2[q] = t * t if r == 0 else a2[q] + t * t
                if r % 7 == 6:
                    ts.append(_token(a1 + a2))
            s1, s2 = a1[0] + a1[1], a2[0] + a2[1]
            m1 = jnp.sum(s1, axis=0, keepdims=True) * (1.0 / D)
            m2 = jnp.sum(s2, axis=0, keepdims=True) * (1.0 / D)
            st[i, 0, :, cs] = x0 + m1
            rs = jnp.broadcast_to(jax.lax.rsqrt(jnp.maximum(m2 - m1 * m1, 0.0) + 1e-5), (8, 128))
            st[i, 1, :, cs] = rs
            return ts + [_token([rs])]

        return staged([functools.partial(job, c) for c in range(TM // 128)], 5)

    RAW = (1, 7, 8, 2)

    def raw_x(i, q, t, r):
        return x2.at[i, RAW[2 * (q // 2) + t // 2], RAW[2 * (q % 2) + t % 2], span(r, 8)]

    def norm_x(i, rs=range(7)):
        def job(q, r, e):
            us = []
            for t in range(4):
                cs = slice(128 * t, 128 * t + 128)
                u = _split(ld(_pk(xr[i + zero[0], span(7 * q + r, 16), cs]), e))
                us.append(_join(*[(v - st[i, 0, :, cs]) * st[i, 1, :, cs] for v in u]))
                raw_x(i, q, t, r)[...] = us[-1]
            return _token(us)

        return [functools.partial(job, q, r) for q in range(4) for r in rs]

    def prep_tok(dst, i, part, rs=range(7)):
        def job(a, r, e):
            u, z = {}, [[[None] * 4 for _ in range(4)] for _ in range(2)]
            for g in XC[a][:2]:
                for n in range(4):
                    q, t = 2 * (g // 2) + n // 2, 2 * (g % 2) + n % 2
                    u[RAW[n]] = ld(raw_x(i, q, t, r)[...] if dst is x2 else _pk(yr[i, BW * q + 16 * r:BW * q + 16 * r + 16, 128 * t:128 * t + 128]), e)
                    z[0][q][t], z[1][q][t] = _split(u[RAW[n]])
            us = []
            for b, t in enumerate(zip(*[_comb2(XC, t, a) for t in z])):
                if a in RAW and b in RAW:
                    if dst is y2:
                        dst[i, a, b, span(r, 8), :] = u[b]
                else:
                    us.append(_join(*t))
                    dst[i, a, b, span(r, 8), :] = us[-1]
            return _token(us)

        return [functools.partial(job, a, r) for a in [PA1[k][1] for k in (ORDO[:4], ORDO[4:])[part]] for r in rs]

    def prep_x(i, part):
        return prep_tok(x2, i, part)

    def prep_y(i, part):
        return prep_tok(y2, i, part)

    def half(ref, i, k, c):
        return jnp.concatenate([ref[i, k, n, 0:GW] for n in ((1, 8), (7, 2))[c]], 0)

    def one(ref, i, k):
        return jnp.concatenate([half(ref, i, k, c) for c in range(2)], 1)

    def xn_tile(i):
        return _up(_unblock(*[one(x2, i, k) for k in (1, 7, 8, 2)]))

    def slot(s):
        return (wnk, wtk, s - SK) if isinstance(s, int) and s >= SK else (wn, wt, s)

    def prep_wn(s, o=None):
        n, _, q = slot(s if o is None else o)
        src = wqkv.at[:, 2 * D:2 * D + TF] if isinstance(s, int) and s == SK + 2 else wraw.at[s]

        def job(r, e):
            zc = _raw_comb(_scomb, quad(src, r, 0, HF, e))
            for k, t in enumerate(zc):
                n[q, k, 8 * r:8 * r + 8, :] = t
            return _token(zc[0:1] + zc[3:])

        return [functools.partial(job, r) for r in range(HD // 16)]

    def prep_wt(s, o=None):
        n, t, q = slot(s)

        def job(k, e):
            u = _pk(_up(ld(n[q, k], e)).T)
            t[q if o is None else o, k] = u
            return _token([u[:, 0:128]])

        return [functools.partial(job, k) for k in range(7)]

    def staged(jobs, n=7):
        def part(job, box, a, e):
            if a == 0:
                box.extend(job(e))
            return box[a]

        return [functools.partial(part, job, box, a) for job, box in [(t, []) for t in jobs] for a in range(n)]

    def prep_gu(j, ns=range(49)):
        js = j if isinstance(j, int) else jnp.minimum(j, NJ - 1)
        low = jax.lax.broadcasted_iota(i32, (8, 128), 1) < 64

        def job(r, e):
            z = [[], []]
            for q in range(4):
                rows = slice(BW * q + 16 * r, BW * q + 16 * r + 16)
                blk = []
                for h in range(2):
                    g, u = [ld(_pk(wraw[3 * js + m, rows, 128 * h:128 * h + 128]), e) for m in range(2)]
                    blk += [jnp.where(low, g, pltpu.roll(u, 64, 1)), jnp.where(low, pltpu.roll(g, 64, 1), u)]
                for n in range(2):
                    z[n].append([_split(t)[n] for t in blk])
            out = []
            for a in range(7):
                for b, t in enumerate(zip(*[_comb2(SC, t, a) for t in z])):
                    out.append(_join(*t))
                    wn2[j & 1, a, b, 8 * r:8 * r + 8, :] = out[-1]
            return [_token(out[7 * a:7 * a + 7]) for a in range(7)]

        def job_t(a, b, e):
            u = _pk(_up(ld(wn2[j & 1, a, b, 0:GW], e)).T)
            wt2[j & 1, a, b] = u
            return _token([u])

        return staged([functools.partial(job, r) for r in range(7)]), [functools.partial(job_t, n // 7, n % 7) for n in ns]

    def prep_d(j, rs=range(4)):
        js = j if isinstance(j, int) else jnp.minimum(j, NJ - 1)

        def job_t(q, h, e):
            u = _pk(_up(ld(_pk(wraw[3 * js + 2, BW * q:BW * q + BW, 128 * h:128 * h + 128]), e)).T)
            wdT[q, 64 * h:64 * h + 64] = u
            return _token([u])

        def job(r, e):
            z = [[_split(ld(wdT[q, span(4 * t + r, 8)], e)) for t in range(4)] for q in range(4)]
            out = []
            for a in range(7):
                for b, t in enumerate(zip(*[_comb2(SC, [[t[n] for t in row] for row in z], a) for n in range(2)])):
                    out.append(_join(*t))
                    wd2[j & 1, a, b, span(r, 8), :] = out[-1]
            return [_token(out[7 * a:7 * a + 7]) for a in range(7)]

        return [functools.partial(job_t, q, h) for q in range(4) for h in range(2)], staged([functools.partial(job, r) for r in rs])

    def finish_dw(j):
        low = jax.lax.broadcasted_iota(i32, (8, 128), 1) < 64

        def job_gu(r, e):
            z = _post_2(_post3, [[pw2[a, b, 16 * r:16 * r + 16, :] for b in range(7)] for a in range(7)])
            for q in range(4):
                u = [_pk(t.astype(bf16)) for t in z[q]]
                for h in range(2):
                    s0, s1 = u[2 * h], u[2 * h + 1]
                    rows, cs = slice(BW * q + 16 * r, BW * q + 16 * r + 16), slice(128 * h, 128 * h + 128)
                    sw[j, 0, rows, cs] = _up(jnp.where(low, s0, pltpu.roll(s1, 64, 1)))
                    sw[j, 1, rows, cs] = _up(jnp.where(low, pltpu.roll(s0, 64, 1), s1))

        def job(r, e):
            c11, c12, c21, c22 = _post3([pw[2, k, 16 * r:16 * r + 16, :] for k in range(7)])
            sw[j, 2, 16 * r:16 * r + 16, :] = jnp.concatenate([c11, c12], 1).astype(bf16)
            sw[j, 2, HD + 16 * r:HD + 16 * r + 16, :] = jnp.concatenate([c21, c22], 1).astype(bf16)

        return [functools.partial(job_gu, r) for r in range(7)] + [functools.partial(job, r) for r in range(HD // 16)]

    def fx(t, e):
        return t if e is None else pltpu.bitcast(ld(pltpu.bitcast(t, u32), e), f32)

    def gelu(act, out, n, p, r, e):
        ps = [[g and g[p][r:r + GS] for g in t] for t in act]
        for t in ps:
            t[(0, 2, 1, 0)[n]] = fx(t[(0, 2, 1, 0)[n]], e)
        out[r // GS] = _gelu_fb(*[_post1z(t, n) for t in ps])
        return _token(out[r // GS])

    def deal(host, name, jobs, lag, lo, hi):
        slots = host.setdefault(name, {})
        for q, job in enumerate(jobs):
            slots.setdefault(lo + q * (hi - lo) // len(jobs), []).append((job, lag))

    def ffn_step(i, j, first_chunk, host, pre, held=()):
        cnt = {}
        idn, jd = i, j & 1

        def at(name):
            q = cnt[name] = cnt.get(name, -1) + 1
            if (name, q) in pre:
                pre[name, q]()
            return host.get(name, {}).pop(q, [])

        def done(q, r):
            t = _token(r)
            host.setdefault("a" if q < 147 else "b", {}).setdefault(q % 147, []).append((lambda e: t, None))

        act, res = [[None] * 7 for _ in range(3)], [None] * 4
        for q1, k1 in enumerate(ORDO):
            a1, b1 = PA1[k1]
            for m in range(3):
                p = [None] * 7
                for k2 in ORD1:
                    a2, b2 = PA1[k2]
                    w = wd2[jd, a1, a2] if m == 2 else wt2[jd, a1, a2, 32 * m:32 * m + 32]
                    p[k2] = mm(pin(w, at("a")), _up((y2 if m == 2 else x2)[idn, b1, b2, 0:GW]))
                act[m][k1] = [_post1n(p, n) for n in range(4)]
                if PINI is not None and q1 < QI:
                    done(21 * q1 + 7 * m + 7 + PINI, act[m][k1])
            if q1 in FINO:
                n = FINO[q1]
                res[n] = [None] * 4
                lo, hi = PING[q1]
                for q, p in enumerate(PORD):
                    res[n][p] = [None] * (64 // GS)
                    for r in range(0, 64, GS):
                        job = functools.partial(gelu, act, res[n][p], n, p, r)
                        if held or n != 3 or q1 < 5:
                            d = 21 * q1 + 21 + lo + (hi - lo) * (64 * q + r) // 256
                            d = d if d < 147 else 147 + (d - 147) // 2
                            host.setdefault("a" if d < 147 else "b", {}).setdefault(d % 147, []).append((job, GL[d >= 147]))
                        else:
                            job(None)

        def zq(r, t, m):
            return jnp.concatenate([u[m] for u in res[2 * (r // 2) + t // 2][2 * (r % 2) + t % 2]], 0)

        @functools.cache
        def dc(k):
            e = entry(DL)
            z = [[None] * 4 for _ in range(4)]
            for n, g in enumerate(SC[k][:2]):
                for r in range(2 * (g // 2), 2 * (g // 2) + 2):
                    for t in range(2 * (g % 2), 2 * (g % 2) + 2):
                        z[r][t] = fx(jnp.concatenate([zq(r, t, 1), zq(r, t, 2)], 0), None if n else e)
            parts = [_comb2(SC, [[t if t is None else t[r:r + SL] for t in row] for row in z], k) for r in range(0, 128, SL)]
            return _cast([jnp.concatenate(t, 0) for t in zip(*parts)])

        @functools.cache
        def hc(c, k):
            e = entry(DL)
            z = [None] * 4
            for n, g in enumerate(SC[k][:2]):
                z[g] = fx(jnp.concatenate([zq(2 * (g // 2) + r, 2 * (g % 2) + c, 0) for r in range(2)], 0), None if n else e)
            return _pick(SC[k], z).astype(bf16)

        def b2(k1, at):
            a1, b1 = PA2[k1]
            for k2 in KORD:
                a2, b2 = PA2[k2]
                t = mm(pin(wn2[j & 1, a1, a2, 0:GW], at("b")), dc(b1)[b2])
                if first_chunk:
                    px2[i, k1, k2, 0:BW] = t
                else:
                    px2[i, k1, k2, 0:BW] += t
            for c in range(NC):
                cs = slice(c * 128, (c + 1) * 128)
                t = mm(pin(wn[j, a1], at("b")), hc(c, b1))
                if first_chunk:
                    po[i, k1, :, cs] = t
                else:
                    po[i, k1, :, cs] += t

        def b3(k1, at):
            a1, b1 = PA3[k1]
            for k2, (a2, b2) in enumerate(PA3):
                t = mm(pin(x2[i, a1, a2, 0:GW], at("b")), dc(b1)[b2], NT)
                if i == 0:
                    pw2[k1, k2, 0:BW] = t
                else:
                    pw2[k1, k2, 0:BW] += t
            t = mm(pin(half(y2, i, a1, 0), at("b")), hc(0, b1), NT) + mm(pin(half(y2, i, a1, 1), at("b")), hc(1, b1), NT)
            if i == 0:
                pw[2, k1] = t
            else:
                pw[2, k1] += t

        for f in held:
            f(at)
        if i == NI - 1:
            order = [(b3, 4), (b3, 2), (b3, 6), (b2, 4), (b3, 0), (b3, 1), (b3, 3), (b3, 5), None] + [(b2, k) for k in (6, 2, 0, 1, 3, 5)]
        else:
            order = [(b2, 4), (b2, 6), (b2, 2), (b3, 4)] + [(b2, k) for k in (0, 1, 3, 5)] + [(b3, k) for k in (2, 6, 0, 1, 3, 5)]
        nh = 0 if i == NI - 1 else HOLD
        for t in order[:len(order) - nh]:
            if t is None:
                run(finish_dw(j))
            else:
                t[0](t[1], at)
        return [functools.partial(*t) for t in order[len(order) - nh:]]

    def att_t():
        def job(lo, n, src, e):
            u = _up(ld(_pk(wqkv[:, src:src + 128]), e)).T if n == 128 else wqkv[:, src:src + n].T
            wT[lo:lo + n, :] = u
            return _token([_pk(u)[:, 0:384]])

        return [functools.partial(job, 128 * n, 128, 128 * n) for n in range(7)] + [
            functools.partial(job, 2 * D, 128, 2 * D + 256), functools.partial(job, 2 * D + 128, 64, 2 * D + 384)]

    def att_phi():
        w3[...] = wphi[...].astype(f32).reshape(D, DH)
        for h in range(H):
            w2[DH * h:DH * (h + 1), :] = w3[pl.ds(h, DH, stride=H), :]
        e112 = _e_rows(0, BW)
        m112 = _head_match((BW, BW), 0, 0, 0)
        for p in range(4):
            pcs[p] = jnp.where(m112, _dot(e112, w2[BW * p:BW * p + BW, :].astype(bf16), NT), 0.0).astype(bf16)

    def att_fold_k():
        for p in range(4):
            tail = wT[2 * D + 128 + 16 * p:2 * D + 144 + 16 * p, :]
            t = jnp.concatenate([_dot(pcs[p], wT[D + BW * p:D + BW * p + BW, :]).astype(bf16), tail], 0)
            wraw[SK + p // 2, 0:D, 128 * (p % 2):128 * (p % 2) + 128] = t.T

    def att_qo(p):
        rows, lanes, z16 = span(p, BW), span(p & 1, 128), jnp.zeros((16, D), bf16)
        t = _dot(pcs[p], wT[rows, :]).astype(bf16)
        wpqT[rows, :] = t
        wraw[SQ[0] + 2 * (p >> 1), 0:D, lanes] = jnp.concatenate([t, z16], 0).T
        wraw[SO[0] + 2 * (p >> 1), 0:D, lanes] = jnp.concatenate([wo[rows, :], z16], 0).T

    zero[0] = jnp.min(jax.lax.broadcasted_iota(i32, (8, 128), 1).astype(f32)).astype(i32)
    first = [cp_x(0, 0), cp_w(0, 0, 1), cp_w(0, 1, 1), cp_w(0, 2, 1), cp_dy(0, 2)]
    grp = [[cp_x(1, 3), cp_dy(1, 3)],
           [cp_x(2, 4), cp_dy(2, 4), cp(wqkv_h, wqkv, 4), cp(wphi_h, wphi, 4), cp_x(3, 4), cp_dy(3, 4)] + [cp_w(1, m, 4) for m in range(3)],
           [cp(wo_h, wo, 5)] + [cp_w(j, m, 5) for j in range(2, NJ) for m in range(3)]]
    for c in first + grp[0] + grp[1][0:2]:
        c.start()
    first[0].wait()
    run(stats_x(0))

    def x0_body(r, carry):
        run(norm_x(0, [r]) + prep_tok(x2, 0, 0, [r]) + prep_tok(x2, 0, 1, [r]))
        return carry

    jax.lax.fori_loop(0, 7, x0_body, 0)
    for c in first[1:4]:
        c.wait()
    (gu, gu0), dd = prep_gu(0, [7 * PA1[a][0] + PA1[b][0] for a in ORDO for b in ORD1]), prep_d(0)
    run(dd[0] + gu + dd[1] + prep_wn(2, 0) + gu0[0:T0])
    for c in grp[1][2:]:
        c.start()
    first[4].wait()

    def interleave(a, b):
        return [t for p in zip(a, b) for t in p]

    def wait_all(cs, nxt=()):
        for c in nxt:
            c.start()
        for c in cs:
            c.wait()

    held = ()
    gu, dd = prep_gu(1), prep_d(1)
    for i in range(NI):
        host, pre = {}, {}
        o = 9 * HOLD * (i > 0)
        if i < NI - 1:
            lo, hi = F0W[i], 126 + o - 9 * HOLD
            if i < 2:
                pre["b", lo] = functools.partial(wait_all, *grp[i:2 * i + 1])
            m1 = 72 + o - WB
            deal(host, "b", stats_x(i + 1), None, lo + 6, lo + 38)
            deal(host, "b", prep_y(i + 1, 0)[0:YS], 12, lo + 20, m1)
            deal(host, "b", norm_x(i + 1) + prep_y(i + 1, 0)[YS:] + prep_x(i + 1, 0), 12, m1, hi)
        if i == 0:
            deal(host, "a", prep_y(0, 0) + prep_y(0, 1), None, 1, Y0)
            deal(host, "a", gu0[T0:], 30, T1, T2)
        else:
            deal(host, "a", interleave(prep_x(i, 1), prep_y(i, 1)), 20, 4, AH)
        if i == 1:
            deal(host, "b", att_t(), LT, 88, 124)
        if i == 2:
            pre["a", 0] = att_phi
            pre["b", 9] = att_fold_k
            deal(host, "b", dd[0], LT, 10, 40)
            deal(host, "b", gu[0][0:GA], 16, 50, 84)
        if i == 3:
            deal(host, "b", gu[0][GA:], 16, 20, 52)
            deal(host, "b", prep_wn(SK + 2) + prep_wn(SK) + prep_wn(SK + 1), 12, W0, 132)
            deal(host, "b", prep_wt(SK + 2) + prep_wt(SK), LT, 124, 134)
            deal(host, "b", prep_wt(SK + 1), LT, 134, 143)
        held = ffn_step(i, 0, True, host, pre, held)
    for c in cp_dw(0):
        c.start()
    wait_all(grp[2])

    def group_rows(c4, g, pitch):
        p = g // 2
        r, h = pitch * (p // 2) + GW * (g % 2), p % 2
        return jnp.concatenate([c4[2 * h][r:r + GW], c4[2 * h + 1][r:r + GW]], 1)

    def p1_body(i, carry):
        def prods(n, c):
            p = [None] * 7
            for k in ORD1:
                a, b = PA1[k]
                p[k] = _dot(_up(wtk[n, a]), _up(half(x2, i, b, c)))
            return _post1(p)

        vt = {}
        for c in range(NC):
            for n in range(2):
                k4 = prods(n, c)
                for q in (2, 1, 3, 0):
                    p, t = 2 * n + q // 2, c + 2 * (q % 2)
                    vt[p, t] = k4[q][BW:128]
                    for g in range(2):
                        a, b = _dual_softmax(k4[q][GW * g:GW * (g + 1)])
                        phik[i, 2 * p + g, :, 128 * t:128 * t + 128] = jnp.concatenate(a + b, axis=0)
        att_qo(i)
        s = jnp.where(i == 0, 5, jnp.where(i < 3, SQ[0] - 1 + i, SO[1]))
        o = jnp.where(i == 0, 1, NJ + i)
        run(prep_wn(s, o) + prep_wt(o, i) + prep_d(1, [i])[1] + prep_gu(1, [12 * i + q for q in range(13)])[1])
        v4 = [prods(2, c) for c in range(NC)]
        v2 = _dot(wT[2 * D:2 * D + 128, :], xn_tile(i))
        vv = jnp.concatenate([jnp.concatenate([v4[t % 2][2 * h + t // 2] for t in range(4)], 1) for h in range(2)] + [v2]
                             + [jnp.concatenate([vt[p, t] for t in range(4)], 1) for p in range(4)], 0)
        ones = jnp.ones((8, TM), f32)
        for g in range(NG):
            va = jnp.concatenate([vv[GW * g:GW * (g + 1)], ones], axis=0).astype(bf16)
            vta[i, g] = _pk(va)
            kv[g] = jnp.where(i > 0, kv[g], 0.0) + _dot(va, phik[i, g].astype(bf16), NT)
        return carry

    jax.lax.fori_loop(0, NI, p1_body, 0)

    def finish_kv(src):
        m = _kv_mask()
        for g in range(NG):
            a = jnp.where(m, src[g], 0.0)
            kvm[g] = a.astype(bf16)
            kvmT[g] = a.T.astype(bf16)


    def f_body(j, carry):
        hist.clear()
        held = ()
        for i in range(NI):
            host = {}
            gu, dd = prep_gu(j + 1), prep_d(j + 1)
            o = 9 * HOLD * (i > 0)
            if i < 2:
                deal(host, "b", gu[0][(0, 21)[i]:(21, 49)[i]], 16, 80 + o, 126 + o - 9 * HOLD)
            if i == 0:
                deal(host, "b", dd[0], LT, 40 + o, 72 + o)
            if i == 2:
                deal(host, "b", gu[1], LT, 40 + o, 126)
                deal(host, "b", prep_wn(3 * j + 5, j + 1), 12, 76 + o, 126)
            if i == 3:
                deal(host, "b", dd[1], 12, 92 + o, 120 + o)
            held = ffn_step(i, j, False, host, {}, held)
        for c in cp_dw(j):
            c.start()
        return carry

    jax.lax.fori_loop(1, NJ, f_body, 0)
    finish_kv(kv)
    cp_keep = [cp(wn.at[NJ - 1, 0, 0:8], wn.at[0, 0, 0:8], 7)]
    cp_keep += [cp(t.at[1, 0, 0, 0:8], t.at[0, 0, 0, 0:8], 7) for t in (wn2, wt2, wd2)]
    for c in cp_keep:
        c.start()

    def p2_body(i, carry):
        def lhs(s, a):
            return _up(jnp.concatenate([wt[s[0], a, 0:GW], wt[s[1], a, 0:GW]], 0))

        pq = _dot(wpqT[...], xn_tile(i))
        do = _post1([_dot(lhs((2, 3), a), _up(one(y2, i, b))) for a, b in PA1])
        low = jax.lax.broadcasted_iota(i32, (8, TM), 0) < 4
        ab, phi, na = [], [], []
        for g in range(NG):
            a, b = _dual_softmax(pq[GW * g:GW * (g + 1)])
            ab.append((a, b))
            phi.append(jnp.concatenate(a + b, axis=0).astype(bf16))
            na.append(_slabs(_dot(kvm[g], phi[g]), 8))
        o_rows, dp_rows = [], []
        for g in range(NG):
            e = 1.0 / (na[g][7] + 1e-6)
            er = pltpu.roll(e, 4, 0)
            ra = jnp.where(low, e, er)
            rb = jnp.where(low, er, e)
            rr = [ra, ra, ra, e, rb, rb, rb]
            o = [n * q for n, q in zip(na[g][:7], rr)]
            dn = [d * q for d, q in zip(_slabs(group_rows(do, g, BW), 7), rr)]
            tt = [p * q for p, q in zip(dn, o)]
            sa = tt[0] + tt[1] + tt[2]
            sb = tt[4] + tt[5] + tt[6]
            ex = jnp.where(low, sa, sb) + pltpu.roll(jnp.where(low, sb, sa), 4, 0) + tt[3]
            dna = jnp.concatenate(dn + [-ex], axis=0).astype(bf16)
            dphi = _dot(kvmT[g], dna)
            dkv[g] = jnp.where(i > 0, dkv[g], 0.0) + _dot(dna, phi[g], NT)
            o_rows += o
            dp_rows += _dual_softmax_bwd(ab[g][0], ab[g][1], dphi)

        def combos(rows):
            return [_cast(_scomb(*_blocks(jnp.concatenate(rows[28 * s:28 * s + 28], 0)))) for s in range(2)]

        def back(s, a, z, b):
            return _dot(_up(wn[s[0], a])[:, 0:BW], z[0][b]) + _dot(_up(wn[s[1], a])[:, 0:BW], z[1][b])

        oc, dc = combos(o_rows), combos(dp_rows)
        res = _post2([po[i, k] + back((NJ + 2, NJ + 3), a, oc, b) for k, (a, b) in enumerate(PA2)])
        sout[i] = (xr[i].astype(f32) + _unblock(*res)).astype(bf16)
        cp_out(i).start()
        for k, (a, b) in enumerate(PA3):
            pa[k] = jnp.where(i > 0, pa[k], 0.0) + _dot(jnp.concatenate([oc[0][b], oc[1][b]], 0), _up(one(y2, i, a)), NT)
        for k, (a, b) in enumerate(PA2):
            px[i, k] = _unblock(*_post2([px2[i, k, n, 0:BW] for n in range(7)])) + back((NJ + 1, NJ), a, dc, b)
        for k, (a, b) in enumerate(PA3):
            for s in range(2):
                pg[s, k] = jnp.where(i > 0, pg[s, k], 0.0) + _dot(_up(one(x2, i, a)), dc[s][b], NT)
        return carry

    jax.lax.fori_loop(0, NI, p2_body, 0)
    finish_kv(dkv)
    for s in range(2):
        c4 = [t.astype(bf16) for t in _post3([pa[k, BW * s:BW * s + BW, :] for k in range(7)])]
        for h in range(2):
            swo[BW * (2 * s + h):BW * (2 * s + h + 1), :] = jnp.concatenate([c4[h], c4[2 + h]], 1)
    cp_datt[4].start()
    for s in range(2):
        c4 = _post3([pg[s, k] for k in range(7)])
        for h in range(2):
            p = 2 * s + h
            g = jnp.concatenate([c4[h], c4[2 + h]], 0).astype(bf16)
            sqkv[:, BW * p:BW * p + BW] = _dot(g, pcs[p]).astype(bf16)
            rq[p] = _dot(wT[BW * p:BW * p + BW, :], g)
    cp_datt[0].start()

    def ln_rows(i, t, r, e):
        dn = [dnb[t, pl.ds(16 * r + q, 8, stride=2), :] for q in range(2)]
        k = (1, 7, 8, 2)[2 * (r // 14) + t // 2]
        return dn, _split(ld(x2[i, k, (1, 7, 8, 2)[2 * (r % 14 // 7) + t % 2], 8 * (r % 7):8 * (r % 7) + 8], e))

    def ln_stats(i, t, e):
        a1, a2 = [None] * 2, [None] * 2
        for r in range(D // 16):
            for q, (d, x) in enumerate(zip(*ln_rows(i, t, r, e))):
                a1[q] = d if r == 0 else a1[q] + d
                a2[q] = d * x if r == 0 else a2[q] + d * x
        ms = [jnp.broadcast_to(jnp.sum(a[0] + a[1], axis=0, keepdims=True) * (1.0 / D), (8, 128)) for a in (a1, a2)]
        for q in range(2):
            lnm[t, q] = ms[q]
        return _token(ms)

    def ln_out(i, t):
        cs = slice(128 * t, 128 * t + 128)

        def job(r, e):
            dn, xf = ln_rows(i, t, r, e)
            ys = _split(_pk(yr[i, 16 * r:16 * r + 16, cs]))
            o = [y + st[i, 1, :, cs] * (d - lnm[t, 0] - x * lnm[t, 1]) for d, x, y in zip(dn, xf, ys)]
            u = _join(*o)
            sdx[i, 16 * r:16 * r + 16, cs] = _up(u)
            return u

        return [fuse([functools.partial(job, r) for r in range(q, q + 2)]) for q in range(0, D // 16, 2)]

    def p3_body(i, carry):
        hist.clear()
        dc, dr = [], [None] * 4
        for c in range(NC):
            dk, dv = {}, {}
            for g in (0, 2, 1, 3, 4, 6, 5, 7):
                for t in (c, c + 2):
                    cs = slice(128 * t, 128 * t + 128)
                    ab = _slabs(phik[i, g, :, cs], 14)
                    dk[g, t] = _dual_softmax_bwd(ab[:7], ab[7:], _dot(kvmT[g], _up(vta[i, g, :, cs])))
            for g in range(NG):
                for t in (c, c + 2):
                    dv[g, t] = _dot(kvm[g], phik[i, g, :, 128 * t:128 * t + 128].astype(bf16))[0:GW]
            z = []
            for h in range(2):
                for t in (c, c + 2):
                    v = jnp.concatenate([dv[g, t] for g in range(NG)], 0)
                    z.append(jnp.concatenate(dk[2 * h, t] + dk[2 * h + 1, t] + [v[384 + 16 * h:400 + 16 * h]] + dk[4 + 2 * h, t]
                                             + dk[5 + 2 * h, t] + [v[416 + 16 * h:432 + 16 * h], v[128 * h:128 * h + 128]], 0))
                    dr[t] = v[256:384].astype(bf16)
            dc.append(_cast(_scomb(*z)))
        host = {}
        for c in range(NC):
            cs = slice(c * 128, (c + 1) * 128)
            jobs = host.get("n", [()] * 14)
            rem = [mm(wqkv[:, 2 * D + 256:2 * D + 384], dr[t]) for t in (c, c + 2)]
            m = [None] * 7
            for q, k in enumerate(ORD2):
                a, b = PA2[k]
                m[k] = px[i, k, :, cs] + mm(pin(jnp.concatenate([wnk[n, a] for n in range(3)], 1), jobs[2 * q]), dc[c][b])
            c4 = _post2(m)
            for q, t in enumerate((c, c + 2)):
                dnb[t, 0:D] = jnp.concatenate([c4[q], c4[2 + q]], 0) + rem[q]
            if c == 0:
                spread(host, "n", [functools.partial(ln_stats, i, 0)], 3, 4, 5)
                spread(host, "n", [functools.partial(ln_stats, i, 2)], 3, 8, 9)
        spread(host, "g", ln_out(i, 0) + ln_out(i, 2), 2, 0, 6)
        spread(host, "g", [functools.partial(ln_stats, i, 1)], 2, 3, 4)
        spread(host, "g", [functools.partial(ln_stats, i, 3)], 2, 5, 6)
        spread(host, "g", ln_out(i, 1) + ln_out(i, 3), 2, 6, 12)
        for k, (a, b) in enumerate(PA3):
            t = sum(mm(pin(half(x2, i, a, c), host["g"][2 * k + c]), dc[c][b], NT) for c in range(NC))
            for q in range(3):
                pw[q, k] = jnp.where(i > 0, pw[q, k], 0.0) + t[:, 128 * q:128 * q + 128]
        cp_dx(i).start()
        grem[...] = jnp.where(i > 0, grem[...], 0.0) + _dot(xn_tile(i), jnp.concatenate(dr, 1), NT)
        return carry

    jax.lax.fori_loop(0, NI, p3_body, 0)

    sqkv[:, 2 * D:2 * D + 256] = _unblock(*_post3([pw[2, k] for k in range(7)])).astype(bf16)
    sqkv[:, 2 * D + 256:2 * D + 384] = grem[...].astype(bf16)
    gk = []
    for s in range(2):
        c4 = _post3([pw[s, k] for k in range(7)])
        for h in range(2):
            p = 2 * s + h
            g = jnp.concatenate([c4[h], c4[2 + h]], 0).astype(bf16)
            sqkv[:, 2 * D + 384 + 16 * p:2 * D + 400 + 16 * p] = g[:, BW:128]
            gk.append(g[:, 0:BW])
    cp_datt[1].start()
    for p in range(4):
        sqkv[:, D + BW * p:D + BW * p + BW] = _dot(gk[p], pcs[p]).astype(bf16)
    cp_datt[2].start()
    e112 = _e_rows(0, BW)
    m112 = _head_match((BW, BW), 1, 0, 0)
    for p in range(4):
        rr = rq[p] + _dot(wT[D + BW * p:D + BW * p + BW, :], gk[p])
        w2[BW * p:BW * p + BW, :] = _dot(jnp.where(m112, rr, 0.0).astype(bf16), e112)
    for h in range(H):
        w3[pl.ds(h, DH, stride=H), :] = w2[DH * h:DH * (h + 1), :]
    sphi[...] = w3[...].reshape(DH, H, DH).astype(bf16)
    cp_datt[3].start()

    for j in range(NJ):
        for c in cp_dw(j):
            c.wait()
    for i in range(NI):
        cp_out(i).wait()
        cp_dx(i).wait()
    for c in cp_datt + cp_keep:
        c.wait()


@jax.jit
def pallas_parallel_sum__linear_kernel_hedgehog__glu_gated_geglu__prompt_kernel(
    A_x: jax.Array,
    A_wqkv: jax.Array,
    A_w_phi: jax.Array,
    A_wo: jax.Array,
    B_x: jax.Array,
    B_w_gate: jax.Array,
    B_w_up: jax.Array,
    B_w_down: jax.Array,
    grad_out: jax.Array,
):
    V = pltpu.VMEM
    scratch = [
        V((NI, D, TM), bf16), V((NI, D, TM), bf16),
        V((NI, 2, 8, TM), f32),
        V((NS, 512, TF), bf16),
        V((NJ + 4, 8, HD // 2, HF), u32), V((4, 8, HF // 2, HD), u32),
        V((3, 8, HD // 2, HF), u32), V((3, 8, HF // 2, HD), u32),
        V((NI, 9, 9, 64, 128), u32), V((NI, 7, 9, 64, 128), u32),
        V((2, 7, 7, 64, 128), u32), V((2, 7, 7, 64, BW), u32), V((2, 7, 7, 32, BW), u32),
        V((4, 128, BW), u32), V((NI, 7, 7, 128, 128), f32), V((7, 7, 128, 128), f32),
        V((NI, 8, HD, HM), f32), V((NI, 8, HD, HM), f32),
        V((3, 8, HD, HF), f32), V((NJ, 3, 512, TF), bf16),
        V((D, 3 * D), bf16), V((DH, H, DH), bf16), V((D, D), bf16),
        V((2 * D + 192, D), bf16), V((D, D), bf16), V((4, BW, BW), bf16),
        V((D, DH), f32), V((D, DH), f32),
        V((NI, NG, BW, TM), f32), V((NI, NG, 32, TM), u32),
        V((NG, 64, 2 * GW), f32), V((NG, 64, 2 * GW), f32),
        V((NG, 64, 2 * GW), bf16), V((NG, 2 * GW, 64), bf16),
        V((4, 512, 128), f32), V((4, 2, 8, 128), f32), V((2, 8, HD, BW), f32), V((8, HD, HD), f32), V((D, 128), f32), V((4, BW, BW), f32),
        V((NI, D, TM), bf16), V((NI, D, TM), bf16), V((D, 3 * D), bf16), V((DH, H, DH), bf16), V((D, D), bf16),
        pltpu.SMEM((1,), i32),
        pltpu.SemaphoreType.DMA((NSEM,)),
    ]
    args = (A_x[0].T, A_wqkv, A_w_phi.transpose(1, 0, 2), A_wo, B_w_gate, B_w_up, B_w_down.T, grad_out[0].T)
    out_shape = tuple(jax.ShapeDtypeStruct(args[k].shape, bf16) for k in (0, 0, 1, 2, 3, 4, 5, 6))
    hbm = pl.BlockSpec(memory_space=pltpu.HBM)
    out, dx, dwqkv, dwphi, dwo, dwg, dwu, dwd = pl.pallas_call(
        _kernel,
        out_shape=out_shape,
        in_specs=[hbm] * len(args),
        out_specs=tuple([hbm] * len(out_shape)),
        scratch_shapes=scratch,
        compiler_params=pltpu.CompilerParams(vmem_limit_bytes=120 * 1024 * 1024),
        name="hedgehog_geglu",
    )(*args)
    return (out.T[None], dx.T[None], dwqkv, dwphi.transpose(1, 0, 2), dwo, dwg, dwu, dwd.T)
```
